```python
import os as _os
_os.environ.setdefault("JAX_PLATFORMS", "cpu")
import jax
import jax.numpy as jnp

def _softmax(x, axis=-1):
    return jax.nn.softmax(x, axis=axis)
def _gelu(x):
    return jax.nn.gelu(x, approximate=True)
def _silu(x):
    return jax.nn.silu(x)
def _sigmoid(x):
    return jax.nn.sigmoid(x)
def _layernorm(x, axis=-1, eps=1e-5):
    m = jnp.mean(x, axis=axis, keepdims=True)
    v = jnp.var(x, axis=axis, keepdims=True)
    return (x - m) / jnp.sqrt(v + eps)
def _scatter_add(tgt, idx, src, axis=0):
    return tgt.at[idx].add(src)
def _segment_sum(src, seg, n):
    return jax.ops.segment_sum(src, seg, n)
class _Rng:
    def __init__(self, key):
        self._k = key
    def _next(self):
        self._k, sub = jax.random.split(self._k)
        return sub
    def normal(self, shape):
        return jax.random.normal(self._next(), shape, dtype=jnp.bfloat16)
    def randint(self, lo, hi, shape):
        return jax.random.randint(self._next(), shape, lo, hi, dtype=jnp.int32)
    def uniform(self, shape, lo=0.0, hi=1.0):
        return jax.random.uniform(self._next(), shape, jnp.bfloat16, lo, hi)
    def permutation(self, n):
        return jax.random.permutation(self._next(), n)


kernel_name = 'gated_mix__sliding_block_cached__swiglu_ffn__decode'

def setup_inputs():
    _rng = _Rng(jax.random.key(int.from_bytes(__import__("os").urandom(4), "little")))
    _w = (lambda a: (lambda t: t.astype(jnp.bfloat16) if jnp.issubdtype(t.dtype, jnp.floating) else t)(jnp.asarray(a)))
    def _A_setup():
        B, Sq, D = 1, 1, 512
        Hq, Hkv, Sk, Dh = 32, 32, 32768, 128
        assert Hq % Hkv == 0, (Hq, Hkv)
        return {
            "x": _w((lambda *s: _rng.normal(s) * 0.05)(B, Sq, D)),
            "k_cache": _w((lambda *s: _rng.normal(s) * 3.2)(B, Hkv, Sk, Dh)),
            "v_cache": _w((lambda *s: _rng.normal(s) * 1.6)(B, Hkv, Sk, Dh)),
            "wq": _w((lambda *s: _rng.normal(s) * 3.2)(D, Hq * Dh) * (D ** -0.5)),
            "wo": _w((lambda *s: _rng.normal(s) * 1.6)(Hq * Dh, D) * ((Hq * Dh) ** -0.5)),
        }
    _A_in = _A_setup()

    def _B_setup():
        B, S, D, F = 1, 1, 512, 1376
        return {
            "x": _w((lambda *s: _rng.normal(s) * 0.05)(B, S, D)),
            "w_gate": _w((lambda *s: _rng.normal(s) * 0.1)(D, F)),
            "w_up": _w((lambda *s: _rng.normal(s) * 0.1)(D, F)),
            "w_down": _w((lambda *s: _rng.normal(s) * 0.1)(F, D)),
        }
    _B_in = _B_setup()

    return {
        "A_x": _A_in["x"],
        "A_k_cache": _A_in["k_cache"],
        "A_v_cache": _A_in["v_cache"],
        "A_wq": _A_in["wq"],
        "A_wo": _A_in["wo"],
        "B_x": _B_in["x"],
        "B_w_gate": _B_in["w_gate"],
        "B_w_up": _B_in["w_up"],
        "B_w_down": _B_in["w_down"],
        "gate_w": _w((lambda *s: _rng.normal(s) * 0.05)(512) * 16.0),
    }

def reference(A_x, A_k_cache, A_v_cache, A_wq, A_wo, B_x, B_w_gate, B_w_up, B_w_down, gate_w):
    def _A_ref(x, k_cache, v_cache, wq, wo):
        B, Sq, D = x.shape
        Hq, Dh = 32, 128
        Hkv, Sk = k_cache.shape[1], k_cache.shape[2]
        W = min(4096, max(256, Sk // 4))
        rep = Hq // Hkv
        q = (lambda x, *d: x.transpose(*d))((x @ wq).reshape(B, Sq, Hq, Dh), 0, 2, 1, 3)
        k = jnp.repeat(k_cache[:, :, Sk - W:, :], rep, axis=1)
        v = jnp.repeat(v_cache[:, :, Sk - W:, :], rep, axis=1)
        scores = jnp.einsum("bhqd,bhkd->bhqk", q, k) * (Dh ** -0.5)
        p = _softmax(scores, axis=-1)
        o = jnp.einsum("bhqk,bhkd->bhqd", p, v)
        return (lambda x, *d: x.transpose(*d))(o, 0, 2, 1, 3).reshape(B, Sq, Hq * Dh) @ wo

    def _B_ref(x, w_gate, w_up, w_down):
        g = _silu(x @ w_gate)
        u = x @ w_up
        return (g * u) @ w_down

    x = A_x
    g = _sigmoid((x * gate_w).sum(-1, keepdims=True))
    a = _A_ref(x, A_k_cache, A_v_cache, A_wq, A_wo)
    b = _B_ref(x, B_w_gate, B_w_up, B_w_down)
    return g * a + (1 - g) * b
```

```python
import jax
import jax.numpy as jnp
from jax import lax
import jax.experimental.pallas as pl
import jax.experimental.pallas.tpu as pltpu

_DH = 128
_NT = (((1,), (1,)), ((), ()))
_DEPTH = 2


@jax.jit
def pallas_gated_mix__sliding_block_cached__swiglu_ffn__decode_kernel(
    A_x: jax.Array,
    A_k_cache: jax.Array,
    A_v_cache: jax.Array,
    A_wq: jax.Array,
    A_wo: jax.Array,
    B_x: jax.Array,
    B_w_gate: jax.Array,
    B_w_up: jax.Array,
    B_w_down: jax.Array,
    gate_w: jax.Array,
):
    del B_x
    D = A_x.shape[-1]
    H, SK = A_k_cache.shape[1], A_k_cache.shape[2]
    W = min(4096, max(256, SK // 4))
    F = B_w_gate.shape[1]
    f32, bf16 = jnp.float32, jnp.bfloat16
    depth, DH, NT = _DEPTH, _DH, _NT

    def kern(x_h, k_h, v_h, wq_h, wo_h, wg_h, wu_h, wd_h, gw_h, o_ref,
             x_v, gw_v, k_v, v_v, wq_v, wo_v, wg_v, wu_v, wd_v, q_s, o_s, kv_sem, w_sem):
        def kv_copy(h, t):
            s, d = ((k_h, k_v), (v_h, v_v))[t]
            return pltpu.make_async_copy(s.at[0, h, pl.ds(SK - W, W)], d.at[h], kv_sem.at[t, h % depth])

        c_wq = pltpu.make_async_copy(wq_h, wq_v, w_sem.at[0])
        c_x = pltpu.make_async_copy(x_h, x_v, w_sem.at[1])
        c_gw = pltpu.make_async_copy(gw_h, gw_v, w_sem.at[2])
        c_wg = pltpu.make_async_copy(wg_h, wg_v, w_sem.at[3])
        c_wu = pltpu.make_async_copy(wu_h, wu_v, w_sem.at[4])
        c_wo = pltpu.make_async_copy(wo_h, wo_v, w_sem.at[5])
        c_wd = pltpu.make_async_copy(wd_h, wd_v, w_sem.at[6])
        c_wq.start()
        c_x.start()
        c_gw.start()
        for h in range(depth):
            kv_copy(h, 0).start()
            kv_copy(h, 1).start()
        c_x.wait()
        c_gw.wait()
        x1 = x_v[0].astype(f32)
        gate = jax.nn.sigmoid(
            jnp.sum(x1 * gw_v[...].astype(f32).reshape(1, D), axis=-1, keepdims=True))
        x8 = jnp.broadcast_to(x1, (8, D)).astype(bf16)
        c_wq.wait()
        q = jnp.dot(x8, wq_v[...], preferred_element_type=f32)
        for h in range(H):
            q_s[h] = q[:, h * DH:(h + 1) * DH]

        def body(h, c):
            kv_copy(h, 0).wait()
            s = lax.dot_general(q_s[h].astype(bf16), k_v[h], NT, preferred_element_type=f32)
            s = s * (DH ** -0.5)
            m = jnp.max(s, axis=-1, keepdims=True)
            e = jnp.exp(s - m)
            l = jnp.sum(e, axis=-1, keepdims=True)
            kv_copy(h, 1).wait()

            @pl.when(h + depth < H)
            def _():
                kv_copy(h + depth, 0).start()
                kv_copy(h + depth, 1).start()

            @pl.when(h + depth == H)
            def _():
                c_wg.start()
                c_wu.start()
                c_wo.start()
                c_wd.start()
            o = jnp.dot(e.astype(bf16), v_v[h], preferred_element_type=f32)
            o_s[h] = o / l
            return c

        lax.fori_loop(0, H, body, 0)
        c_wg.wait()
        c_wu.wait()
        g = lax.dot_general(x8, wg_v[...], NT, preferred_element_type=f32)
        u = lax.dot_general(x8, wu_v[...], NT, preferred_element_type=f32)
        hid = (g * jax.nn.sigmoid(g) * u).astype(bf16)
        o_all = jnp.concatenate([o_s[h] for h in range(H)], axis=-1).astype(bf16)
        c_wo.wait()
        a = jnp.dot(o_all, wo_v[...], preferred_element_type=f32)
        c_wd.wait()
        b = jnp.dot(hid, wd_v[...], preferred_element_type=f32)
        res = gate * a[0:1] + (1.0 - gate) * b[0:1]
        o_ref[0] = res.astype(o_ref.dtype)

    hb = pl.BlockSpec(memory_space=pltpu.HBM)
    return pl.pallas_call(
        kern,
        out_shape=jax.ShapeDtypeStruct(A_x.shape, A_x.dtype),
        in_specs=[hb] * 9,
        scratch_shapes=[
            pltpu.VMEM(A_x.shape, bf16), pltpu.VMEM(gate_w.shape, bf16),
            pltpu.VMEM((H, W, DH), bf16), pltpu.VMEM((H, W, DH), bf16),
            pltpu.VMEM(A_wq.shape, bf16), pltpu.VMEM(A_wo.shape, bf16),
            pltpu.VMEM((F, D), bf16), pltpu.VMEM((F, D), bf16), pltpu.VMEM((F, D), bf16),
            pltpu.VMEM((H, 8, DH), f32), pltpu.VMEM((H, 8, DH), f32),
            pltpu.SemaphoreType.DMA((2, depth)), pltpu.SemaphoreType.DMA((7,)),
        ],
        compiler_params=pltpu.CompilerParams(vmem_limit_bytes=100 * 1024 * 1024),
        name="gated_mix_decode",
    )(A_x, A_k_cache, A_v_cache, A_wq, A_wo, B_w_gate.T, B_w_up.T, B_w_down, gate_w)
```

```python
import jax
import jax.numpy as jnp
from jax import lax
import jax.experimental.pallas as pl
import jax.experimental.pallas.tpu as pltpu

_DH = 128
_HG = 8
_BLK = 512
_LAG = 2
_KV_HEADS, _KV_ROWS = 2, 64
_WQ_ROWS, _WQ_COLS = 16, 1024
_W_ROWS = 32
_STREAMS = 8
_WO_LAST = 2
_NT = (((1,), (1,)), ((), ()))


def _start(src, dst, sem, queue):
    pltpu.make_async_copy(src, dst, sem).start(priority=queue % 2)


def _wait(buf, sem):
    pltpu.make_async_copy(buf, buf, sem).wait()


def _loop(n, body):
    def step(i, carry):
        body(i)
        return carry

    lax.fori_loop(0, n, step, 0)


def _rows(start, size):
    return pl.ds(pl.multiple_of(start, size), size)


def _kernel(x_h, k_h, v_h, wq_h, wo_h, wg_h, wu_h, wd_h, gw_h, out_ref,
            x_v, gw_v, k_v, v_v, wq_v, wo_v, wg_v, wu_v, wd_v, q_s, o_s):
    f32, bf16 = jnp.float32, jnp.bfloat16
    heads, window, _ = k_v.shape
    first_pos = k_h.shape[2] - window
    d_model, d_ff = x_v.shape[-1], wg_v.shape[0]
    blocks = window // _BLK
    steps = heads // _HG * blocks
    wo_rounds = heads // _STREAMS
    wo_pieces = [(c * _STREAMS, (c + 1) * _STREAMS) for c in range(wo_rounds - 1)]
    wo_pieces += [(heads - _STREAMS, heads - _WO_LAST), (heads - _WO_LAST, heads)]
    ffn = ((wg_h, wg_v), (wu_h, wu_v), (wd_h, wd_v))

    def group_and_block(t):
        return lax.shift_right_logical(t, blocks.bit_length() - 1), t & (blocks - 1)

    def run(k_sem, v_sem, in_sem, ffn_sem, wo_sem):
        def start_wq(j):
            for c in range(heads * _DH // _WQ_COLS):
                for s in range(_STREAMS):
                    idx = (_rows(s * (d_model // _STREAMS) + j * _WQ_ROWS, _WQ_ROWS),
                           pl.ds(c * _WQ_COLS, _WQ_COLS))
                    _start(wq_h.at[idx], wq_v.at[idx], in_sem.at[0], s)

        def start_kv(t):
            g, r = group_and_block(t)

            def body(j):
                pos = r * _BLK + j * _KV_ROWS
                src, dst = _rows(first_pos + pos, _KV_ROWS), _rows(pos, _KV_ROWS)
                for h in range(0, _HG, _KV_HEADS):
                    hs = pl.ds(g * _HG + h, _KV_HEADS)
                    _start(k_h.at[0, hs, src], k_v.at[hs, dst], k_sem.at[t], 0)
                    _start(v_h.at[0, hs, src], v_v.at[hs, dst], v_sem.at[t], 1)

            _loop(_BLK // _KV_ROWS, body)

        def start_ffn():
            def one(u, queue):
                rows = _rows(u * _W_ROWS, _W_ROWS)
                for n, (src, dst) in enumerate(ffn):
                    _start(src.at[rows], dst.at[rows], ffn_sem.at[n], queue + n)

            def two(j):
                one(2 * j, 0)
                one(2 * j + 1, 1)

            units = d_ff // _W_ROWS
            _loop(units // 2, two)
            if units % 2:
                one(units - 1, 0)

        def start_wo():
            for p, (lo, hi) in enumerate(wo_pieces):
                def body(j, p=p, lo=lo, hi=hi):
                    for slot in range(lo, hi):
                        head = slot % _STREAMS * wo_rounds + slot // _STREAMS
                        queue = 1 if hi == heads else slot + 1
                        _start(wo_h.at[_rows(head * _DH + j * _W_ROWS, _W_ROWS)],
                               wo_v.at[_rows(slot * _DH + j * _W_ROWS, _W_ROWS)],
                               wo_sem.at[p], queue)

                _loop(_DH // _W_ROWS, body)

        x_copy = pltpu.make_async_copy(x_h, x_v, in_sem.at[1])
        gw_copy = pltpu.make_async_copy(gw_h, gw_v, in_sem.at[2])
        _loop(d_model // _STREAMS // _WQ_ROWS, start_wq)
        x_copy.start(priority=0)
        gw_copy.start(priority=1)
        _loop(_LAG, start_kv)
        x_copy.wait()
        gw_copy.wait()
        _wait(wq_v, in_sem.at[0])

        x = x_v[0].astype(f32)
        x_rows = jnp.broadcast_to(x, (_HG, d_model)).astype(bf16)
        q = jnp.dot(x_rows, wq_v[...], preferred_element_type=f32)
        row = lax.broadcasted_iota(jnp.int32, (_HG, _DH), 0)
        for g in range(heads // _HG):
            q_g = q[:, g * _HG * _DH:(g * _HG + 1) * _DH]
            for i in range(1, _HG):
                h = g * _HG + i
                q_g = jnp.where(row == i, q[:, h * _DH:(h + 1) * _DH], q_g)
            q_s[g] = q_g

        def attend(t, carry):
            @pl.when(t < steps - _LAG)
            def _():
                start_kv(jnp.minimum(t + _LAG, steps - 1))

            pl.when(t == steps - _LAG)(start_ffn)

            g, r = group_and_block(t)
            pos = _rows(r * _BLK, _BLK)
            _wait(k_v.at[pl.ds(g * _HG, _HG), pos], k_sem.at[t])
            _wait(v_v.at[pl.ds(g * _HG, _HG), pos], v_sem.at[t])

            m_old = jnp.where(r == 0, -jnp.inf, carry[0])
            l_old = jnp.where(r == 0, 0.0, carry[1])
            acc = jnp.where(r == 0, 0.0, carry[2])

            q_g = q_s[g].astype(bf16)
            s_row = lax.broadcasted_iota(jnp.int32, (_HG, _BLK), 0)
            s = None
            for i in range(_HG):
                s_i = lax.dot_general(q_g, k_v[g * _HG + i, pos, :], _NT,
                                      preferred_element_type=f32)
                s = s_i if s is None else jnp.where(s_row == i, s_i, s)
            s = s * _DH ** -0.5

            m_new = jnp.maximum(m_old, jnp.max(s, axis=-1, keepdims=True))
            shift = jnp.where(m_new == -jnp.inf, 0.0, m_new)
            alpha = jnp.exp(m_old - shift)
            p = jnp.exp(s - shift)
            l_new = alpha * l_old + jnp.sum(p, axis=-1, keepdims=True)

            p = p.astype(bf16)
            pv = None
            for i in range(_HG):
                pv_i = jnp.dot(p, v_v[g * _HG + i, pos, :], preferred_element_type=f32)
                pv = pv_i if pv is None else jnp.where(row == i, pv_i, pv)
            acc = alpha * acc + pv
            o_s[g] = acc / l_new
            return m_new, l_new, acc

        stat = jnp.zeros((_HG, 1), f32)
        lax.fori_loop(0, steps, attend, (stat, stat, jnp.zeros((_HG, _DH), f32)))
        start_wo()

        gate_w = gw_v[...].astype(f32).reshape(1, d_model)
        gate = jax.nn.sigmoid(jnp.sum(x * gate_w, axis=-1, keepdims=True))

        for n, (_, dst) in enumerate(ffn):
            _wait(dst, ffn_sem.at[n])
        g_proj = lax.dot_general(x_rows, wg_v[...], _NT, preferred_element_type=f32)
        u_proj = lax.dot_general(x_rows, wu_v[...], _NT, preferred_element_type=f32)
        hidden = (g_proj * jax.nn.sigmoid(g_proj) * u_proj).astype(bf16)
        out = (1.0 - gate) * jnp.dot(hidden, wd_v[...], preferred_element_type=f32)

        for p, (lo, hi) in enumerate(wo_pieces):
            piece_heads = [s % _STREAMS * wo_rounds + s // _STREAMS for s in range(lo, hi)]
            attn = jnp.concatenate(
                [jnp.broadcast_to(o_s[h // _HG, pl.ds(h % _HG, 1), :], (_HG, _DH))
                 for h in piece_heads], axis=-1).astype(bf16)
            piece = wo_v.at[pl.ds(lo * _DH, (hi - lo) * _DH)]
            _wait(piece, wo_sem.at[p])
            out = out + gate * jnp.dot(attn, piece[...], preferred_element_type=f32)
        out_ref[0] = out[0:1].astype(out_ref.dtype)

    dma = pltpu.SemaphoreType.DMA
    pl.run_scoped(run, dma((steps,)), dma((steps,)), dma((3,)), dma((3,)),
                  dma((len(wo_pieces),)))


@jax.jit
def pallas_gated_mix__sliding_block_cached__swiglu_ffn__decode_kernel(
    A_x: jax.Array,
    A_k_cache: jax.Array,
    A_v_cache: jax.Array,
    A_wq: jax.Array,
    A_wo: jax.Array,
    B_x: jax.Array,
    B_w_gate: jax.Array,
    B_w_up: jax.Array,
    B_w_down: jax.Array,
    gate_w: jax.Array,
):
    del B_x
    _, heads, seq, head_dim = A_k_cache.shape
    window = min(4096, max(256, seq // 4))
    blocks = window // _BLK
    d_ff, d_model = B_w_down.shape
    assert A_x.shape == (1, 1, d_model) and A_wq.shape == (d_model, heads * _DH)
    assert head_dim == _DH and heads % _HG == 0 and heads % _STREAMS == 0
    assert window == blocks * _BLK and blocks & (blocks - 1) == 0
    assert (seq - window) % _KV_ROWS == 0 and d_ff % _W_ROWS == 0
    assert d_model % (_STREAMS * _WQ_ROWS) == 0

    def vmem(a, shape=None):
        return pltpu.VMEM(shape or a.shape, a.dtype)

    per_head = pltpu.VMEM((heads // _HG, _HG, _DH), jnp.float32)
    w_gate_t, w_up_t = B_w_gate.T, B_w_up.T
    return pl.pallas_call(
        _kernel,
        out_shape=jax.ShapeDtypeStruct(A_x.shape, A_x.dtype),
        in_specs=[pl.BlockSpec(memory_space=pltpu.MemorySpace.HBM)] * 9,
        scratch_shapes=[
            vmem(A_x), vmem(gate_w),
            vmem(A_k_cache, (heads, window, _DH)), vmem(A_v_cache, (heads, window, _DH)),
            vmem(A_wq), vmem(A_wo), vmem(w_gate_t), vmem(w_up_t), vmem(B_w_down),
            per_head, per_head,
        ],
        compiler_params=pltpu.CompilerParams(vmem_limit_bytes=100 * 1024 * 1024),
        name="gated_mix_decode",
    )(A_x, A_k_cache, A_v_cache, A_wq, A_wo, w_gate_t, w_up_t, B_w_down, gate_w)
```

```python
import jax
import jax.numpy as jnp
from jax import lax
import jax.experimental.pallas as pl
import jax.experimental.pallas.tpu as pltpu

_DH = 128
_HG = 8
_BLK = 512
_LAG = 3
_KV_HEADS, _KV_ROWS = 2, 64
_WQ_ROWS, _WQ_COLS = 16, 1024
_W_ROWS = 32
_STREAMS = 8
_WO_PIECES = (8, 8, 8, 6, 2)
_WO_LATE = 1
_NT = (((1,), (1,)), ((), ()))


def _start(src, dst, sem, priority):
    pltpu.make_async_copy(src, dst, sem).start(priority=priority)


def _wait(buf, sem):
    pltpu.make_async_copy(buf, buf, sem).wait()


def _loop(lo, hi, body):
    def step(i, carry):
        body(i)
        return carry

    lax.fori_loop(lo, hi, step, 0)


def _rows(start, size):
    return pl.ds(pl.multiple_of(start, size), size)


def _kernel(x_h, k_h, v_h, wq_h, wo_h, wg_h, wu_h, wd_h, gw_h, out_ref,
            x_v, gw_v, k_v, v_v, wq_v, wo_v, wg_v, wu_v, wd_v, q_s, o_s):
    f32, bf16 = jnp.float32, jnp.bfloat16
    heads, window, _ = k_v.shape
    first_pos = k_h.shape[2] - window
    d_model, d_ff = x_v.shape[-1], wg_v.shape[0]
    blocks = window // _BLK
    steps = heads // _HG * blocks
    ffn = ((wg_h, wg_v), (wu_h, wu_v), (wd_h, wd_v))
    wo_head = [i % _STREAMS * (heads // _STREAMS) + i // _STREAMS for i in range(heads)]
    wo_slots = [range(sum(_WO_PIECES[:p]), sum(_WO_PIECES[:p + 1]))
                for p in range(len(_WO_PIECES))]

    def group_and_block(t):
        return lax.shift_right_logical(t, blocks.bit_length() - 1), t & (blocks - 1)

    def run(in_sem, k_sem, v_sem, wo_sem):
        wq_sem = in_sem.at[len(ffn)]
        x_copy = pltpu.make_async_copy(x_h, x_v, in_sem.at[len(ffn) + 1])
        gw_copy = pltpu.make_async_copy(gw_h, gw_v, in_sem.at[len(ffn) + 2])

        def start_wq_and_ffn():
            wq_tiles = [(pl.ds(s * (d_model // _STREAMS) + r, _WQ_ROWS), pl.ds(c, _WQ_COLS))
                        for r in range(0, d_model // _STREAMS, _WQ_ROWS)
                        for c in range(0, heads * _DH, _WQ_COLS)
                        for s in range(_STREAMS)]
            ffn_tiles = [(n, pl.ds(r, _W_ROWS))
                         for r in range(0, d_ff, _W_ROWS) for n in range(len(ffn))]
            for i in range(max(len(wq_tiles), len(ffn_tiles))):
                if i < len(ffn_tiles):
                    n, rows = ffn_tiles[i]
                    _start(ffn[n][0].at[rows], ffn[n][1].at[rows], in_sem.at[n], 0)
                if i < len(wq_tiles):
                    _start(wq_h.at[wq_tiles[i]], wq_v.at[wq_tiles[i]], wq_sem, 1)

        def start_kv(t):
            g, r = group_and_block(t)

            def body(j):
                pos = r * _BLK + j * _KV_ROWS
                src, dst = _rows(first_pos + pos, _KV_ROWS), _rows(pos, _KV_ROWS)
                for h in range(0, _HG, _KV_HEADS):
                    hs = pl.ds(g * _HG + h, _KV_HEADS)
                    _start(k_h.at[0, hs, src], k_v.at[hs, dst], k_sem.at[t], 0)
                    _start(v_h.at[0, hs, src], v_v.at[hs, dst], v_sem.at[t], 1)

            _loop(0, _BLK // _KV_ROWS, body)

        def start_wo(pieces):
            for p in pieces:
                def body(j, p=p):
                    for slot in wo_slots[p]:
                        _start(wo_h.at[_rows(wo_head[slot] * _DH + j * _W_ROWS, _W_ROWS)],
                               wo_v.at[_rows(slot * _DH + j * _W_ROWS, _W_ROWS)],
                               wo_sem.at[p],
                               1 if p >= len(wo_slots) - _WO_LATE else slot % 2)

                _loop(0, _DH // _W_ROWS, body)

        start_wq_and_ffn()
        x_copy.start(priority=1)
        gw_copy.start(priority=1)
        _loop(0, _LAG - 1, start_kv)

        x_copy.wait()
        _wait(wq_v, wq_sem)
        x = x_v[0].astype(f32)
        x_rows = jnp.broadcast_to(x, (_HG, d_model)).astype(bf16)
        q = jnp.dot(x_rows, wq_v[...], preferred_element_type=f32)
        row = lax.broadcasted_iota(jnp.int32, (_HG, _DH), 0)
        for g in range(heads // _HG):
            q_g = q[:, g * _HG * _DH:(g * _HG + 1) * _DH]
            for i in range(1, _HG):
                h = g * _HG + i
                q_g = jnp.where(row == i, q[:, h * _DH:(h + 1) * _DH], q_g)
            q_s[g] = q_g
        _loop(_LAG - 1, _LAG, start_kv)

        gw_copy.wait()
        for n, (_, dst) in enumerate(ffn):
            _wait(dst, in_sem.at[n])
        gate_w = gw_v[...].astype(f32).reshape(1, d_model)
        gate = jax.nn.sigmoid(jnp.sum(x * gate_w, axis=-1, keepdims=True))
        g_proj = lax.dot_general(x_rows, wg_v[...], _NT, preferred_element_type=f32)
        u_proj = lax.dot_general(x_rows, wu_v[...], _NT, preferred_element_type=f32)
        hidden = (g_proj * jax.nn.sigmoid(g_proj) * u_proj).astype(bf16)
        out = (1.0 - gate) * jnp.dot(hidden, wd_v[...], preferred_element_type=f32)

        def attend(t, carry):
            @pl.when(t < steps - _LAG)
            def _():
                start_kv(jnp.minimum(t + _LAG, steps - 1))

            pl.when(t == steps - _LAG)(lambda: start_wo(range(2)))
            pl.when(t == steps - _LAG + 1)(lambda: start_wo(range(2, len(wo_slots))))

            g, r = group_and_block(t)
            pos = _rows(r * _BLK, _BLK)
            _wait(k_v.at[pl.ds(g * _HG, _HG), pos], k_sem.at[t])
            _wait(v_v.at[pl.ds(g * _HG, _HG), pos], v_sem.at[t])

            m_old = jnp.where(r == 0, -jnp.inf, carry[0])
            l_old = jnp.where(r == 0, 0.0, carry[1])
            acc = jnp.where(r == 0, 0.0, carry[2])

            q_g = q_s[g].astype(bf16)
            s_row = lax.broadcasted_iota(jnp.int32, (_HG, _BLK), 0)
            s = None
            for i in range(_HG):
                s_i = lax.dot_general(q_g, k_v[g * _HG + i, pos, :], _NT,
                                      preferred_element_type=f32)
                s = s_i if s is None else jnp.where(s_row == i, s_i, s)
            s = s * _DH ** -0.5

            m_new = jnp.maximum(m_old, jnp.max(s, axis=-1, keepdims=True))
            shift = jnp.where(m_new == -jnp.inf, 0.0, m_new)
            alpha = jnp.exp(m_old - shift)
            p = jnp.exp(s - shift)
            l_new = alpha * l_old + jnp.sum(p, axis=-1, keepdims=True)

            p = p.astype(bf16)
            pv = None
            for i in range(_HG):
                pv_i = jnp.dot(p, v_v[g * _HG + i, pos, :], preferred_element_type=f32)
                pv = pv_i if pv is None else jnp.where(row == i, pv_i, pv)
            acc = alpha * acc + pv
            o_s[g] = acc / l_new
            return m_new, l_new, acc

        stat = jnp.zeros((_HG, 1), f32)
        lax.fori_loop(0, steps, attend, (stat, stat, jnp.zeros((_HG, _DH), f32)))

        for p, slots in enumerate(wo_slots):
            attn = jnp.concatenate(
                [jnp.broadcast_to(o_s[h // _HG, pl.ds(h % _HG, 1), :], (_HG, _DH))
                 for h in (wo_head[slot] for slot in slots)], axis=-1).astype(bf16)
            rows = pl.ds(slots.start * _DH, len(slots) * _DH)
            _wait(wo_v.at[rows], wo_sem.at[p])
            out = out + gate * jnp.dot(attn, wo_v[rows, :], preferred_element_type=f32)
        out_ref[0] = out[0:1].astype(out_ref.dtype)

    dma = pltpu.SemaphoreType.DMA
    pl.run_scoped(run, dma((len(ffn) + 3,)), dma((steps,)), dma((steps,)),
                  dma((len(wo_slots),)))


@jax.jit
def pallas_gated_mix__sliding_block_cached__swiglu_ffn__decode_kernel(
    A_x: jax.Array,
    A_k_cache: jax.Array,
    A_v_cache: jax.Array,
    A_wq: jax.Array,
    A_wo: jax.Array,
    B_x: jax.Array,
    B_w_gate: jax.Array,
    B_w_up: jax.Array,
    B_w_down: jax.Array,
    gate_w: jax.Array,
):
    del B_x
    _, heads, seq, head_dim = A_k_cache.shape
    window = min(4096, max(256, seq // 4))
    blocks = window // _BLK
    d_ff, d_model = B_w_down.shape
    assert A_x.shape == (1, 1, d_model) and A_wq.shape == (d_model, heads * _DH)
    assert head_dim == _DH and heads == sum(_WO_PIECES)
    assert window == blocks * _BLK and blocks & (blocks - 1) == 0
    assert (seq - window) % _KV_ROWS == 0 and d_ff % _W_ROWS == 0
    assert d_model % (_STREAMS * _WQ_ROWS) == 0

    def vmem(a, shape=None):
        return pltpu.VMEM(shape or a.shape, a.dtype)

    per_head = pltpu.VMEM((heads // _HG, _HG, _DH), jnp.float32)
    w_gate_t, w_up_t = B_w_gate.T, B_w_up.T
    return pl.pallas_call(
        _kernel,
        out_shape=jax.ShapeDtypeStruct(A_x.shape, A_x.dtype),
        in_specs=[pl.BlockSpec(memory_space=pltpu.MemorySpace.HBM)] * 9,
        scratch_shapes=[
            vmem(A_x), vmem(gate_w),
            vmem(A_k_cache, (heads, window, _DH)), vmem(A_v_cache, (heads, window, _DH)),
            vmem(A_wq), vmem(A_wo), vmem(w_gate_t), vmem(w_up_t), vmem(B_w_down),
            per_head, per_head,
        ],
        compiler_params=pltpu.CompilerParams(vmem_limit_bytes=100 * 1024 * 1024),
        name="gated_mix_decode",
    )(A_x, A_k_cache, A_v_cache, A_wq, A_wo, w_gate_t, w_up_t, B_w_down, gate_w)
```
